```python
import os as _os
_os.environ.setdefault("JAX_PLATFORMS", "cpu")
import jax
import jax.numpy as jnp

def _softmax(x, axis=-1):
    return jax.nn.softmax(x, axis=axis)
def _gelu(x):
    return jax.nn.gelu(x, approximate=True)
def _silu(x):
    return jax.nn.silu(x)
def _sigmoid(x):
    return jax.nn.sigmoid(x)
def _layernorm(x, axis=-1, eps=1e-5):
    m = jnp.mean(x, axis=axis, keepdims=True)
    v = jnp.var(x, axis=axis, keepdims=True)
    return (x - m) / jnp.sqrt(v + eps)
def _scatter_add(tgt, idx, src, axis=0):
    return tgt.at[idx].add(src)
def _segment_sum(src, seg, n):
    return jax.ops.segment_sum(src, seg, n)
class _Rng:
    def __init__(self, key):
        self._k = key
    def _next(self):
        self._k, sub = jax.random.split(self._k)
        return sub
    def normal(self, shape):
        return jax.random.normal(self._next(), shape, dtype=jnp.bfloat16)
    def randint(self, lo, hi, shape):
        return jax.random.randint(self._next(), shape, lo, hi, dtype=jnp.int32)
    def uniform(self, shape, lo=0.0, hi=1.0):
        return jax.random.uniform(self._next(), shape, jnp.bfloat16, lo, hi)
    def permutation(self, n):
        return jax.random.permutation(self._next(), n)


kernel_name = 'parallel_sum__ssm_conv_s5__glu_gated_swiglu__prompt'

def setup_inputs():
    _rng = _Rng(jax.random.key(int.from_bytes(__import__("os").urandom(4), "little")))
    _w = (lambda a: (lambda t: t.astype(jnp.bfloat16) if jnp.issubdtype(t.dtype, jnp.floating) else t)(jnp.asarray(a)))
    def _A_setup():
        B, S, D = 1, 2048, 640
        P = D
        Lambda_re = -0.5 * jnp.exp((lambda *s: _rng.normal(s) * 0.4)(P))
        Lambda_im = (lambda *s: _rng.normal(s) * 0.4)(P) * 1.0
        B_re = (lambda *s: _rng.normal(s) * 0.4)(P, D) * (D ** -0.5)
        B_im = (lambda *s: _rng.normal(s) * 0.4)(P, D) * (D ** -0.5)
        C_re = (lambda *s: _rng.normal(s) * 0.4)(D, P) * (P ** -0.5)
        C_im = (lambda *s: _rng.normal(s) * 0.4)(D, P) * (P ** -0.5)
        log_dt = (lambda *s: _rng.normal(s) * 0.4)(P) * 0.3 - 2.0
        Dskip = (lambda *s: _rng.normal(s) * 0.4)(D)
        return {
            "x": _w((lambda *s: _rng.normal(s) * 0.05)(B, S, D)),
            "Lambda_re": _w(Lambda_re),
            "Lambda_im": _w(Lambda_im),
            "B_re": _w(B_re),
            "B_im": _w(B_im),
            "C_re": _w(C_re),
            "C_im": _w(C_im),
            "log_dt": _w(log_dt),
            "Dskip": _w(Dskip),
        }
    _A_in = _A_setup()

    def _B_setup():
        B, S, D, F = 1, 2048, 640, 1728
        return {
            "x": _w((lambda *s: _rng.normal(s) * 0.05)(B, S, D)),
            "w1": _w((lambda *s: _rng.normal(s) * 0.1)(D, F) * (2.0 / D) ** 0.5),
            "w3": _w((lambda *s: _rng.normal(s) * 0.1)(D, F) * (2.0 / D) ** 0.5),
            "w2": _w((lambda *s: _rng.normal(s) * 0.1)(F, D) * (2.0 / F) ** 0.5),
        }
    _B_in = _B_setup()

    return {
        "A_x": _A_in["x"],
        "A_Lambda_re": _A_in["Lambda_re"],
        "A_Lambda_im": _A_in["Lambda_im"],
        "A_B_re": _A_in["B_re"],
        "A_B_im": _A_in["B_im"],
        "A_C_re": _A_in["C_re"],
        "A_C_im": _A_in["C_im"],
        "A_log_dt": _A_in["log_dt"],
        "A_Dskip": _A_in["Dskip"],
        "B_x": _B_in["x"],
        "B_w1": _B_in["w1"],
        "B_w3": _B_in["w3"],
        "B_w2": _B_in["w2"],
    }

def reference(A_x, A_Lambda_re, A_Lambda_im, A_B_re, A_B_im, A_C_re, A_C_im, A_log_dt, A_Dskip, B_x, B_w1, B_w3, B_w2):
    def _A_ref(x, Lambda_re, Lambda_im, B_re, B_im, C_re, C_im, log_dt, Dskip):
        Bsz, L, H = x.shape
        Lam = Lambda_re + 1j * Lambda_im
        Bmat = B_re + 1j * B_im
        Cmat = C_re + 1j * C_im
        dt = jnp.exp(log_dt)
        Lam_bar = jnp.exp(dt * Lam)
        B_bar = ((Lam_bar - 1.0) / Lam)[:, None] * Bmat
        Bu = jnp.einsum("bld,pd->blp", x + 0j, B_bar)
        h = jnp.zeros_like(Bu[:, 0, :])
        hs = []
        for t in range(L):
            h = Lam_bar[None, :] * h + Bu[:, t, :]
            hs.append(h)
        hseq = jnp.stack(hs, 1)
        y = 2.0 * jnp.einsum("blp,dp->bld", hseq, Cmat).real + x * Dskip[None, None, :]
        return y

    def _B_ref(x, w1, w3, w2):
        gate = jnp.einsum("bsd,df->bsf", x, w1)
        up = jnp.einsum("bsd,df->bsf", x, w3)
        h = _silu(gate) * up
        out = jnp.einsum("bsf,fd->bsd", h, w2)
        return out

    x = A_x
    xn = _layernorm(x, axis=-1)
    return x + _A_ref(xn, A_Lambda_re, A_Lambda_im, A_B_re, A_B_im, A_C_re, A_C_im, A_log_dt, A_Dskip) + _B_ref(xn, B_w1, B_w3, B_w2)
```

```python
import functools
import jax
import jax.numpy as jnp
from jax import lax
import jax.experimental.pallas as pl
import jax.experimental.pallas.tpu as pltpu

T = 256
NSEG = 8
SEG = T // NSEG
F32 = jnp.float32
BF16 = jnp.bfloat16


def _cmul(ar, ai, br, bi):
    return ar * br - ai * bi, ar * bi + ai * br


def _nt(a, b):
    return lax.dot_general(a, b, (((1,), (1,)), ((), ())), preferred_element_type=F32)


def _kernel(x_hbm, lre_hbm, lim_hbm, bre_hbm, bim_hbm, cre_hbm, cim_hbm, ldt_hbm, dsk_hbm,
            w1_hbm, w3_hbm, w2_hbm, o_hbm,
            xin, v0, v1, v2, v3, wa, w2, craw, wc, lam, carry, dsk, xp_ref, pin, pout, obuf, res, sems, osem):
    S, D = x_hbm.shape
    P = bre_hbm.shape[0]
    F = w2_hbm.shape[0]
    FM = (F // 128) * 128
    FT = F - FM
    NB = S // T
    NL = D // 128

    def cp(src, dst, k):
        return pltpu.make_async_copy(src, dst, sems.at[k])
    small = [cp(lre_hbm, v0, 0), cp(lim_hbm, v1, 1), cp(ldt_hbm, v2, 2), cp(dsk_hbm, v3, 3)]
    c_x0 = cp(x_hbm.at[pl.ds(0, T)], xin.at[pl.ds(0, T)], 4)
    c_b = [cp(bre_hbm, wa.at[pl.ds(0, P)], 5), cp(bim_hbm, wa.at[pl.ds(P, P)], 6)]
    c_w = [cp(w1_hbm.at[pl.ds(0, FM)], wa.at[pl.ds(2 * P, FM)], 7),
           cp(w3_hbm.at[pl.ds(0, FM)], wa.at[pl.ds(2 * P + FM, FM)], 8),
           cp(w1_hbm.at[pl.ds(FM, FT)], wa.at[pl.ds(2 * P + 2 * FM, FT)], 9),
           cp(w3_hbm.at[pl.ds(FM, FT)], wa.at[pl.ds(2 * P + 2 * FM + FT, FT)], 10)]
    c_x1 = cp(x_hbm.at[pl.ds(T, T)], xin.at[pl.ds(T, T)], 15)
    c_xr = cp(x_hbm.at[pl.ds(2 * T, S - 2 * T)], xin.at[pl.ds(2 * T, S - 2 * T)], 11)
    c_c = [cp(cre_hbm, craw.at[0], 12), cp(cim_hbm, craw.at[1], 13)]
    c_w2 = cp(w2_hbm, w2, 14)

    c_x0.start()
    for c in small + c_b:
        c.start()

    def prep(blk, slot):
        r0 = pl.multiple_of(blk * T, T)
        x = xin[pl.ds(r0, T), :].astype(F32)
        m = jnp.mean(x, axis=-1, keepdims=True)
        xc = x - m
        v = jnp.mean(xc * xc, axis=-1, keepdims=True)
        xn = xc * lax.rsqrt(v + 1e-5)
        res[slot] = x + xn * dsk[0:1, :]
        for c in range(NL):
            for s in range(NSEG):
                pin[c, pl.ds(s * (SEG + 1), SEG), :] = xn[s * SEG:(s + 1) * SEG, 128 * c:128 * c + 128]
        xp_ref[slot] = jnp.concatenate(
            [jnp.concatenate([pin[c, pl.ds(j, NSEG, stride=SEG + 1), :] for j in range(SEG)], axis=0)
             for c in range(NL)], axis=1).astype(BF16)

    for c in small:
        c.wait()
    dsk[...] = jnp.broadcast_to(v3[...].astype(F32).reshape(1, D), (8, D))
    c_x0.wait()
    for c in [c_w[0], c_w[2]]:
        c.start()
    prep(0, 0)
    lre = v0[...].astype(F32).reshape(1, P)
    lim = v1[...].astype(F32).reshape(1, P)
    dt = jnp.exp(v2[...].astype(F32).reshape(1, P)).astype(BF16).astype(F32)
    mag = jnp.exp(dt * lre)
    ar = mag * jnp.cos(dt * lim)
    ai = mag * jnp.sin(dt * lim)
    den = lre * lre + lim * lim
    nr = ar - 1.0
    lam[8] = jnp.broadcast_to(2.0 * (nr * lre + ai * lim) / den, (8, P))
    lam[9] = jnp.broadcast_to(2.0 * (ai * lre - nr * lim) / den, (8, P))
    pr, pi = ar, ai
    lam[0] = jnp.broadcast_to(ar, (8, P))
    lam[1] = jnp.broadcast_to(ai, (8, P))
    n = 1
    while n < SEG:
        pr, pi = _cmul(pr, pi, pr, pi)
        n *= 2
    for k in range(3):
        lam[2 + 2 * k] = jnp.broadcast_to(pr, (8, P))
        lam[3 + 2 * k] = jnp.broadcast_to(pi, (8, P))
        pr, pi = _cmul(pr, pi, pr, pi)
    carry[...] = jnp.zeros(carry.shape, F32)

    def out_copy(blk):
        r0 = pl.multiple_of(blk * T, T)
        return pltpu.make_async_copy(obuf.at[pl.ds(r0, T)], o_hbm.at[pl.ds(r0, T)], osem.at[blk])

    def body(i, first):
        slot = i % 2
        xp = xp_ref[slot]
        if first:
            for c in c_b:
                c.wait()
            c_w[1].start()
            c_w[3].start()
        bur = _nt(xp, wa[0:P, :])
        bui = _nt(xp, wa[P:2 * P, :])
        if first:
            c_w[0].wait()
            c_w2.start()
        ar = lam[0]
        ai = lam[1]
        hr = bur[0:8]
        hi = bui[0:8]
        for j in range(1, SEG):
            tr, ti = _cmul(ar, ai, hr, hi)
            hr = tr + bur[8 * j:8 * j + 8]
            hi = ti + bui[8 * j:8 * j + 8]
        sub = lax.broadcasted_iota(jnp.int32, (8, P), 0)
        sr = jnp.where(sub == 0, carry[0], pltpu.roll(hr, 1, 0))
        si = jnp.where(sub == 0, carry[1], pltpu.roll(hi, 1, 0))
        for k in range(3):
            d = 1 << k
            rr = jnp.where(sub >= d, pltpu.roll(sr, d, 0), 0.0)
            ri = jnp.where(sub >= d, pltpu.roll(si, d, 0), 0.0)
            tr, ti = _cmul(lam[2 + 2 * k], lam[3 + 2 * k], rr, ri)
            sr = sr + tr
            si = si + ti
        hr, hi = sr, si
        hs_r = []
        hs_i = []
        for j in range(SEG):
            tr, ti = _cmul(ar, ai, hr, hi)
            hr = tr + bur[8 * j:8 * j + 8]
            hi = ti + bui[8 * j:8 * j + 8]
            hs_r.append(hr)
            hs_i.append(hi)
        carry[0] = jnp.broadcast_to(hr[7:8], (8, P))
        carry[1] = jnp.broadcast_to(hi[7:8], (8, P))
        hre = jnp.concatenate(hs_r, axis=0).astype(BF16)
        him = jnp.concatenate(hs_i, axis=0).astype(BF16)

        g = _nt(xp, wa[2 * P:2 * P + FM, :])
        if first:
            for c in c_w[1:]:
                c.wait()
            for c in [c_x1] + c_c:
                c.start()
        u = _nt(xp, wa[2 * P + FM:2 * P + 2 * FM, :])
        gu = _nt(xp, wa[2 * P + 2 * FM:, :])
        hh = (g * jax.nn.sigmoid(g) * u).astype(BF16)
        ht = (gu * jax.nn.sigmoid(gu) * pltpu.roll(gu, FT, 1))[:, :FT].astype(BF16)
        if first:
            c_w2.wait()
            c_x1.wait()
            c_xr.start()
            prep(1, 1)
        else:
            prep(jnp.minimum(i + 1, NB - 1), 1 - slot)
        y = jnp.dot(hh, w2[0:FM, :], preferred_element_type=F32)
        y = y + jnp.dot(ht, w2[FM:, :], preferred_element_type=F32)
        if first:
            for c in c_c:
                c.wait()
            cr = lam[8][0:1]
            ci = lam[9][0:1]
            for r in range(0, D, 32):
                c_re = craw[0, r:r + 32].astype(F32)
                c_im = craw[1, r:r + 32].astype(F32)
                wc[r:r + 32, :P] = (c_re * cr - c_im * ci).astype(BF16)
                wc[r:r + 32, P:] = (-(c_re * ci + c_im * cr)).astype(BF16)
        y = y + _nt(hre, wc[:, :P]) + _nt(him, wc[:, P:])
        for c in range(NL):
            for j in range(SEG):
                pout[c, pl.ds(j, NSEG, stride=SEG + 1), :] = y[8 * j:8 * j + 8, 128 * c:128 * c + 128]
        r0 = pl.multiple_of(i * T, T)
        yy = jnp.concatenate(
            [jnp.concatenate([pout[c, pl.ds(s * (SEG + 1), SEG), :] for s in range(NSEG)], axis=0)
             for c in range(NL)], axis=1)
        obuf[pl.ds(r0, T), :] = res[slot] + yy
        out_copy(i).start()
        if first:
            c_xr.wait()

    body(0, True)

    def loop(i, _):
        body(i, False)
        return 0
    lax.fori_loop(1, NB, loop, 0)
    for b in range(NB):
        out_copy(b).wait()


@jax.jit
def pallas_parallel_sum__ssm_conv_s5__glu_gated_swiglu__prompt_kernel(
        A_x, A_Lambda_re, A_Lambda_im, A_B_re, A_B_im, A_C_re, A_C_im, A_log_dt, A_Dskip,
        B_x, B_w1, B_w3, B_w2):
    Bsz, S, D = A_x.shape
    P = A_Lambda_re.shape[0]
    F = B_w1.shape[1]
    x2 = A_x.reshape(S, D)
    hbm = pl.BlockSpec(memory_space=pltpu.HBM)
    out = pl.pallas_call(
        _kernel,
        in_specs=[hbm] * 12,
        out_specs=hbm,
        out_shape=jax.ShapeDtypeStruct((S, D), F32),
        scratch_shapes=[pltpu.VMEM((S, D), BF16),
                        pltpu.VMEM((P,), BF16), pltpu.VMEM((P,), BF16), pltpu.VMEM((P,), BF16), pltpu.VMEM((D,), BF16),
                        pltpu.VMEM((2 * P + 2 * F, D), BF16), pltpu.VMEM((F, D), BF16),
                        pltpu.VMEM((2, D, P), BF16), pltpu.VMEM((D, 2 * P), BF16),
                        pltpu.VMEM((10, 8, P), F32), pltpu.VMEM((2, 8, P), F32), pltpu.VMEM((8, D), F32),
                        pltpu.VMEM((2, T, D), BF16),
                        pltpu.VMEM((D // 128, T + NSEG, 128), F32), pltpu.VMEM((D // 128, T + NSEG, 128), F32),
                        pltpu.VMEM((S, D), F32), pltpu.VMEM((2, T, D), F32),
                        pltpu.SemaphoreType.DMA((16,)), pltpu.SemaphoreType.DMA((S // T,))],
        compiler_params=pltpu.CompilerParams(vmem_limit_bytes=100 * 1024 * 1024),
    )(x2, A_Lambda_re, A_Lambda_im, A_B_re, A_B_im, A_C_re, A_C_im,
      A_log_dt, A_Dskip, B_w1.T, B_w3.T, B_w2)
    return out.reshape(Bsz, S, D)
```
